```python
import os as _os
_os.environ.setdefault("JAX_PLATFORMS", "cpu")
import jax
import jax.numpy as jnp

def _softmax(x, axis=-1):
    return jax.nn.softmax(x, axis=axis)
def _gelu(x):
    return jax.nn.gelu(x, approximate=True)
def _silu(x):
    return jax.nn.silu(x)
def _sigmoid(x):
    return jax.nn.sigmoid(x)
def _layernorm(x, axis=-1, eps=1e-5):
    m = jnp.mean(x, axis=axis, keepdims=True)
    v = jnp.var(x, axis=axis, keepdims=True)
    return (x - m) / jnp.sqrt(v + eps)
def _scatter_add(tgt, idx, src, axis=0):
    return tgt.at[idx].add(src)
def _segment_sum(src, seg, n):
    return jax.ops.segment_sum(src, seg, n)
class _Rng:
    def __init__(self, key):
        self._k = key
    def _next(self):
        self._k, sub = jax.random.split(self._k)
        return sub
    def normal(self, shape):
        return jax.random.normal(self._next(), shape, dtype=jnp.bfloat16)
    def randint(self, lo, hi, shape):
        return jax.random.randint(self._next(), shape, lo, hi, dtype=jnp.int32)
    def uniform(self, shape, lo=0.0, hi=1.0):
        return jax.random.uniform(self._next(), shape, jnp.bfloat16, lo, hi)
    def permutation(self, n):
        return jax.random.permutation(self._next(), n)


kernel_name = 'standalone__gqa_softmax__near_ridge'

def setup_inputs():
    _rng = _Rng(jax.random.key(int.from_bytes(__import__("os").urandom(4), "little")))
    _w = (lambda a: (lambda t: t.astype(jnp.bfloat16) if jnp.issubdtype(t.dtype, jnp.floating) else t)(jnp.asarray(a)))
    B, Hq, Hkv, Sq, Sk, D = 8, 16, 8, 512, 512, 256
    return {
        "q": _w((lambda *s: _rng.normal(s) * 0.4)(B, Hq, Sq, D)),
        "k": _w((lambda *s: _rng.normal(s) * 0.4)(B, Hkv, Sk, D)),
        "v": _w((lambda *s: _rng.normal(s) * 0.05)(B, Hkv, Sk, D)),
    }

def reference(q, k, v):
    B, Hq, Sq, D = q.shape
    Hkv = k.shape[1]
    rep = Hq // Hkv
    k = jnp.repeat(k, rep, axis=1)
    v = jnp.repeat(v, rep, axis=1)
    scale = D ** -0.5
    scores = jnp.einsum("bhqd,bhkd->bhqk", q, k) * scale
    p = _softmax(scores, axis=-1)
    return jnp.einsum("bhqk,bhkd->bhqd", p, v)
```

```python
import math

import jax
import jax.numpy as jnp
from jax import lax
import jax.experimental.pallas as pl
import jax.experimental.pallas.tpu as pltpu

UNROLL = 16
LOOKAHEAD = 4
Q_PIECES = 4
O_PIECES = 4
LATE_WAITS = 3


@jax.jit
def pallas_standalone__gqa_softmax__near_ridge_kernel(
    q: jax.Array,
    k: jax.Array,
    v: jax.Array,
):
    B, Hq, Sq, D = q.shape
    _, Hkv, Sk, _ = k.shape
    G = B * Hkv
    M = (Hq // Hkv) * Sq
    U = math.gcd(G, UNROLL)
    LA = min(LOOKAHEAD, U - 1)
    assert LA >= 1
    HK = Sk // 2
    QR = M // Q_PIECES
    OR = M // O_PIECES
    FIRST_SEMS = 4 + Q_PIECES
    exp2_scale = (D ** -0.5) * math.log2(math.e)

    def kernel(q_hbm, k_hbm, v_hbm, o_hbm, q_buf, k_buf, vo_buf, in_sem, out_sem):

        def fetch(src, dst, g, row, rows, sem):
            return pltpu.make_async_copy(
                src.at[g, pl.ds(row, rows)], dst.at[g, pl.ds(row, rows)], in_sem.at[sem])

        def k_piece(g, j):
            return fetch(k_hbm, k_buf, g, j * HK, HK, j)

        def v_piece(g, j):
            return fetch(v_hbm, vo_buf, g, j * HK, HK, 2 + j)

        def q_piece(g, j):
            return fetch(q_hbm, q_buf, g, j * QR, QR, 4 + j)

        def k_full(g, u):
            return fetch(k_hbm, k_buf, g, 0, Sk, FIRST_SEMS + u)

        def q_full(g, u):
            return fetch(q_hbm, q_buf, g, 0, M, FIRST_SEMS + u)

        def v_full(g, u):
            return fetch(v_hbm, vo_buf, g, 0, Sk, FIRST_SEMS + (u if u > 1 else 0))

        def start_fetch(g, u):
            if u == 0:
                k_piece(g, 0).start()
                for j in range(Q_PIECES // 2):
                    q_piece(g, j).start()
                k_piece(g, 1).start()
                for j in range(Q_PIECES // 2, Q_PIECES):
                    q_piece(g, j).start()
                v_piece(g, 0).start()
                v_piece(g, 1).start()
            else:
                k_full(g, u).start()
                q_full(g, u).start()
                v_full(g, u).start()

        def qk(a, b):
            return lax.dot_general(
                a, b, (((1,), (1,)), ((), ())), preferred_element_type=jnp.float32)

        def first_scores(g):
            def load_q(lo, hi):
                pieces = []
                for j in range(lo, hi):
                    q_piece(g, j).wait()
                    pieces.append(q_buf[g, j * QR:(j + 1) * QR])
                return jnp.concatenate(pieces, axis=0)

            k_piece(g, 0).wait()
            top = load_q(0, Q_PIECES // 2)
            s00 = qk(top, k_buf[g, 0:HK])
            k_piece(g, 1).wait()
            s01 = qk(top, k_buf[g, HK:Sk])
            bottom = load_q(Q_PIECES // 2, Q_PIECES)
            s0 = jnp.concatenate([s00, qk(bottom, k_buf[g, 0:HK])], axis=0)
            s1 = jnp.concatenate([s01, qk(bottom, k_buf[g, HK:Sk])], axis=0)
            return jnp.concatenate([s0, s1], axis=1)

        def group(g, u):
            s = first_scores(g) if u == 0 else qk(q_buf[g], k_buf[g])
            m = jnp.max(s, axis=-1, keepdims=True)
            p = jnp.exp2((s - m) * exp2_scale)
            l = jnp.sum(p, axis=-1, keepdims=True)

            if u == 0:
                v_piece(g, 0).wait()
            elif u == 1:
                v_full(g, u).wait()
            o = jnp.dot(p[:, :HK].astype(v.dtype), vo_buf[g, 0:HK],
                        preferred_element_type=jnp.float32)
            if u == 0:
                v_piece(g, 1).wait()
            o = o + jnp.dot(p[:, HK:].astype(v.dtype), vo_buf[g, HK:Sk],
                            preferred_element_type=jnp.float32)

            r = pltpu.reciprocal(l, approx=True)
            r = r + r * (1.0 - l * r)
            o = (o * r).astype(q.dtype)

            def write(lo, hi):
                vo_buf[g, Sk + lo:Sk + hi] = o[lo:hi]
                pltpu.make_async_copy(
                    vo_buf.at[g, pl.ds(Sk + lo, hi - lo)],
                    o_hbm.at[g, pl.ds(lo, hi - lo)],
                    out_sem.at[0]).start()

            def prefetch():
                if u + LA < U:
                    start_fetch(g + LA, u + LA)
                else:
                    @pl.when(g + LA < G)
                    def _():
                        start_fetch(g + LA, u + LA - U)

            def wait_next():
                k_full(g + 1, u + 1).wait()
                q_full(g + 1, u + 1).wait()
                if u + 1 > 1:
                    v_full(g + 1, u + 1).wait()

            if u == U - 1:
                for j in range(O_PIECES):
                    write(j * OR, (j + 1) * OR)
                prefetch()
            elif u < LATE_WAITS:
                write(0, OR)
                prefetch()
                wait_next()
                write(OR, M)
            else:
                wait_next()
                write(0, M)
                prefetch()

        for g in range(LA):
            start_fetch(g, g)

        @pl.loop(0, G // U)
        def _(it):
            for u in range(U):
                group(it * U + u, u)

        pltpu.make_async_copy(vo_buf.at[:, pl.ds(Sk, M)], o_hbm, out_sem.at[0]).wait()

    out = pl.pallas_call(
        kernel,
        in_specs=[pl.BlockSpec(memory_space=pl.ANY)] * 3,
        out_specs=pl.BlockSpec(memory_space=pl.ANY),
        out_shape=jax.ShapeDtypeStruct((G, M, D), q.dtype),
        scratch_shapes=[
            pltpu.VMEM((G, M, D), q.dtype),
            pltpu.VMEM((G, Sk, D), k.dtype),
            pltpu.VMEM((G, Sk + M, D), v.dtype),
            pltpu.SemaphoreType.DMA((FIRST_SEMS + U,)),
            pltpu.SemaphoreType.DMA((1,)),
        ],
        compiler_params=pltpu.CompilerParams(
            vmem_limit_bytes=120 * 1024 * 1024,
            disable_bounds_checks=True,
            disable_semaphore_checks=True,
            flags={
                "XLA_TPU_FORCE_LP_LLO_SCHEDULER": True,
                "XLA_TPU_RESCHEDULE_DMA_DONES": True,
            },
        ),
    )(q.reshape(G, M, D), k.reshape(G, Sk, D), v.reshape(G, Sk, D))
    return out.reshape(B, Hq, Sq, D)
```

```python
import math

import jax
import jax.numpy as jnp
from jax import lax
import jax.experimental.pallas as pl
import jax.experimental.pallas.tpu as pltpu

UNROLL = 16
LOOKAHEAD = 4
Q_PIECES = 8
O_PIECES = 16
LATE_WAITS = 3


@jax.jit
def pallas_standalone__gqa_softmax__near_ridge_kernel(
    q: jax.Array,
    k: jax.Array,
    v: jax.Array,
):
    B, Hq, Sq, D = q.shape
    _, Hkv, Sk, _ = k.shape
    G = B * Hkv
    M = (Hq // Hkv) * Sq
    U = math.gcd(G, UNROLL)
    LA = min(LOOKAHEAD, U - 1)
    assert LA >= 1 and q.dtype == v.dtype
    HK = Sk // 2
    QR = M // Q_PIECES
    OR = M // O_PIECES
    FIRST_SEMS = 4 + Q_PIECES
    exp2_scale = (D ** -0.5) * math.log2(math.e)

    def kernel(q_hbm, k_hbm, v_hbm, o_hbm, q_buf, k_buf, vo_buf, in_sem, out_sem):

        def fetch(src, dst, g, row, rows, sem):
            return pltpu.make_async_copy(
                src.at[g, pl.ds(row, rows)], dst.at[g, pl.ds(row, rows)], in_sem.at[sem])

        def k_piece(g, j):
            return fetch(k_hbm, k_buf, g, j * HK, HK, j)

        def v_piece(g, j):
            return fetch(v_hbm, vo_buf, g, j * HK, HK, 2 + j)

        def q_piece(g, j):
            return fetch(q_hbm, q_buf, g, j * QR, QR, 4 + j)

        def k_full(g, u):
            return fetch(k_hbm, k_buf, g, 0, Sk, FIRST_SEMS + 3 * (u - 1))

        def q_full(g, u):
            return fetch(q_hbm, q_buf, g, 0, M, FIRST_SEMS + 3 * (u - 1) + 1)

        def v_full(g, u):
            return fetch(v_hbm, vo_buf, g, 0, Sk, FIRST_SEMS + 3 * (u - 1) + 2)

        def start_fetch(g, u):
            if u == 0:
                k_piece(g, 0).start()
                for j in range(Q_PIECES // 2):
                    q_piece(g, j).start()
                k_piece(g, 1).start()
                for j in range(Q_PIECES // 2, Q_PIECES):
                    q_piece(g, j).start()
                v_piece(g, 0).start()
                v_piece(g, 1).start()
            else:
                k_full(g, u).start()
                q_full(g, u).start()
                v_full(g, u).start()

        def qk(a, b):
            return lax.dot_general(
                a, b, (((1,), (1,)), ((), ())), preferred_element_type=jnp.float32)

        def first_scores(g):
            def load_q(lo, hi):
                pieces = []
                for j in range(lo, hi):
                    q_piece(g, j).wait()
                    pieces.append(q_buf[g, j * QR:(j + 1) * QR])
                return jnp.concatenate(pieces, axis=0)

            k_piece(g, 0).wait()
            top = load_q(0, Q_PIECES // 2)
            s00 = qk(top, k_buf[g, 0:HK])
            k_piece(g, 1).wait()
            s01 = qk(top, k_buf[g, HK:Sk])
            bottom = load_q(Q_PIECES // 2, Q_PIECES)
            s0 = jnp.concatenate([s00, qk(bottom, k_buf[g, 0:HK])], axis=0)
            s1 = jnp.concatenate([s01, qk(bottom, k_buf[g, HK:Sk])], axis=0)
            return jnp.concatenate([s0, s1], axis=1)

        def group(g, u):
            s = first_scores(g) if u == 0 else qk(q_buf[g], k_buf[g])
            m = jnp.max(s, axis=-1, keepdims=True)
            p = jnp.exp2((s - m) * exp2_scale)
            l = jnp.sum(p, axis=-1, keepdims=True)

            if u == 0:
                v_piece(g, 0).wait()
            else:
                v_full(g, u).wait()
            o = jnp.dot(p[:, :HK].astype(v.dtype), vo_buf[g, 0:HK],
                        preferred_element_type=jnp.float32)
            if u == 0:
                v_piece(g, 1).wait()
            o = o + jnp.dot(p[:, HK:].astype(v.dtype), vo_buf[g, HK:Sk],
                            preferred_element_type=jnp.float32)

            o = (o * pltpu.reciprocal(l, full_range=False)).astype(q.dtype)

            def write(lo, hi):
                vo_buf[g, Sk + lo:Sk + hi] = o[lo:hi]
                pltpu.make_async_copy(
                    vo_buf.at[g, pl.ds(Sk + lo, hi - lo)],
                    o_hbm.at[g, pl.ds(lo, hi - lo)],
                    out_sem.at[0]).start()

            def prefetch():
                if u + LA < U:
                    start_fetch(g + LA, u + LA)
                else:
                    @pl.when(g + LA < G)
                    def _():
                        start_fetch(g + LA, u + LA - U)

            def wait_next():
                k_full(g + 1, u + 1).wait()
                q_full(g + 1, u + 1).wait()

            if u == U - 1:
                for j in range(O_PIECES):
                    write(j * OR, (j + 1) * OR)
                prefetch()
            elif u < LATE_WAITS:
                write(0, M // 2)
                prefetch()
                wait_next()
                write(M // 2, M)
            else:
                wait_next()
                write(0, M)
                prefetch()

        for g in range(LA):
            start_fetch(g, g)

        @pl.loop(0, G // U)
        def _(it):
            for u in range(U):
                group(it * U + u, u)

        pltpu.make_async_copy(vo_buf.at[:, pl.ds(Sk, M)], o_hbm, out_sem.at[0]).wait()

    out = pl.pallas_call(
        kernel,
        in_specs=[pl.BlockSpec(memory_space=pl.ANY)] * 3,
        out_specs=pl.BlockSpec(memory_space=pl.ANY),
        out_shape=jax.ShapeDtypeStruct((G, M, D), q.dtype),
        scratch_shapes=[
            pltpu.VMEM((G, M, D), q.dtype),
            pltpu.VMEM((G, Sk, D), k.dtype),
            pltpu.VMEM((G, Sk + M, D), v.dtype),
            pltpu.SemaphoreType.DMA((FIRST_SEMS + 3 * (U - 1),)),
            pltpu.SemaphoreType.DMA((1,)),
        ],
        compiler_params=pltpu.CompilerParams(
            vmem_limit_bytes=120 * 1024 * 1024,
            disable_bounds_checks=True,
            disable_semaphore_checks=True,
            flags={
                "XLA_TPU_FORCE_LP_LLO_SCHEDULER": True,
                "XLA_TPU_RESCHEDULE_DMA_DONES": True,
            },
        ),
    )(q.reshape(G, M, D), k.reshape(G, Sk, D), v.reshape(G, Sk, D))
    return out.reshape(B, Hq, Sq, D)
```
